```python
import os as _os
_os.environ.setdefault("JAX_PLATFORMS", "cpu")
import jax
import jax.numpy as jnp

def _softmax(x, axis=-1):
    return jax.nn.softmax(x, axis=axis)
def _gelu(x):
    return jax.nn.gelu(x, approximate=True)
def _silu(x):
    return jax.nn.silu(x)
def _sigmoid(x):
    return jax.nn.sigmoid(x)
def _layernorm(x, axis=-1, eps=1e-5):
    m = jnp.mean(x, axis=axis, keepdims=True)
    v = jnp.var(x, axis=axis, keepdims=True)
    return (x - m) / jnp.sqrt(v + eps)
def _scatter_add(tgt, idx, src, axis=0):
    return tgt.at[idx].add(src)
def _segment_sum(src, seg, n):
    return jax.ops.segment_sum(src, seg, n)
class _Rng:
    def __init__(self, key):
        self._k = key
    def _next(self):
        self._k, sub = jax.random.split(self._k)
        return sub
    def normal(self, shape):
        return jax.random.normal(self._next(), shape, dtype=jnp.bfloat16)
    def randint(self, lo, hi, shape):
        return jax.random.randint(self._next(), shape, lo, hi, dtype=jnp.int32)
    def uniform(self, shape, lo=0.0, hi=1.0):
        return jax.random.uniform(self._next(), shape, jnp.bfloat16, lo, hi)
    def permutation(self, n):
        return jax.random.permutation(self._next(), n)


kernel_name = 'gated_mix__softmax_full_mha__dense_activation_relu__prompt'

def setup_inputs():
    _rng = _Rng(jax.random.key(int.from_bytes(__import__("os").urandom(4), "little")))
    _w = (lambda a: (lambda t: t.astype(jnp.bfloat16) if jnp.issubdtype(t.dtype, jnp.floating) else t)(jnp.asarray(a)))
    def _A_setup():
        B, S, D = 1, 2048, 640
        return {
            "x": _w((lambda *s: _rng.normal(s) * 0.05)(B, S, D)),
            "wqkv": _w((lambda *s: _rng.normal(s) * 0.8)(D, 3 * D)),
            "wo": _w((lambda *s: _rng.normal(s) * 0.05)(D, D)),
        }
    _A_in = _A_setup()

    def _B_setup():
        B, S, D, Dff = 1, 2048, 640, 1536
        return {
            "x": _w((lambda *s: _rng.normal(s) * 0.05)(B, S, D)),
            "w1": _w((lambda *s: _rng.normal(s) * 0.05)(D, Dff)),
            "w2": _w((lambda *s: _rng.normal(s) * 0.05)(Dff, D)),
        }
    _B_in = _B_setup()

    return {
        "A_x": _A_in["x"],
        "A_wqkv": _A_in["wqkv"],
        "A_wo": _A_in["wo"],
        "B_x": _B_in["x"],
        "B_w1": _B_in["w1"],
        "B_w2": _B_in["w2"],
        "gate_w": _w((lambda *s: _rng.normal(s) * 0.05)(640) * 16.0),
    }

def reference(A_x, A_wqkv, A_wo, B_x, B_w1, B_w2, gate_w):
    def _A_ref(x, wqkv, wo):
        B, S, D = x.shape
        H = 32; Dh = D // H
        qkv = (lambda x, *d: x.transpose(*d))((x @ wqkv).reshape(B, S, 3, H, Dh), 2, 0, 3, 1, 4)
        q, k, v = qkv[0], qkv[1], qkv[2]
        scale = Dh ** -0.5
        scores = jnp.einsum("bhqd,bhkd->bhqk", q, k) * scale
        p = _softmax(scores, axis=-1)
        o = jnp.einsum("bhqk,bhkd->bhqd", p, v)
        return (lambda x, *d: x.transpose(*d))(o, 0, 2, 1, 3).reshape(B, S, D) @ wo

    def _B_ref(x, w1, w2):
        h = jnp.einsum("bsd,df->bsf", x, w1)
        zero = jnp.zeros_like(h)
        h = jnp.maximum(h, zero)
        return jnp.einsum("bsf,fd->bsd", h, w2)

    x = A_x
    g = _sigmoid((x * gate_w).sum(-1, keepdims=True))
    a = _A_ref(x, A_wqkv, A_wo)
    b = _B_ref(x, B_w1, B_w2)
    return g * a + (1 - g) * b
```

```python
import functools
import jax
import jax.numpy as jnp
import numpy as np
from jax import lax
import jax.experimental.pallas as pl
import jax.experimental.pallas.tpu as pltpu

S, D, H, DH, DFF = 2048, 640, 32, 20, 1536
LOG2E = 1.4426950408889634
f32, bf16 = jnp.float32, jnp.bfloat16

def make(BQ=512, CK=128):
    NQ = S // BQ
    NC = S // CK

    def kernel(x_ref, wqkv_ref, wo_ref, w1_ref, w2_ref, gw_ref, o_ref,
               kext_ref, vt_ref, qt_ref, sa_ref, sb_ref, ot_ref):
        qi = pl.program_id(0)

        @pl.when(qi == 0)
        def _():
            lane = lax.broadcasted_iota(jnp.int32, (512, 128), 1)
            def kv_body(r, _):
                rows = pl.ds(pl.multiple_of(r * 512, 512), 512)
                xr = x_ref[rows, :]
                k = jnp.dot(xr, wqkv_ref[:, D:2 * D], preferred_element_type=f32)
                for j in range(5):
                    kext_ref[2 * j, rows, :] = k[:, j * 128:(j + 1) * 128].astype(bf16)
                for j in range(4):
                    kext_ref[2 * j + 1, rows, :] = jnp.where(
                        lane >= 64, k[:, j * 128:(j + 1) * 128], k[:, (j + 1) * 128:(j + 2) * 128]).astype(bf16)
                v = jnp.dot(xr, wqkv_ref[:, 2 * D:3 * D], preferred_element_type=f32)
                vt_ref[r] = v.T.astype(bf16)
                return 0
            lax.fori_loop(0, S // 512, kv_body, 0)

        rows = pl.ds(pl.multiple_of(qi * BQ, BQ), BQ)
        xq = x_ref[rows, :]
        q = jnp.dot(xq, wqkv_ref[:, 0:D], preferred_element_type=f32) * (DH ** -0.5 * LOG2E)
        qt_ref[...] = q.T.astype(bf16)
        ot_ref[...] = jnp.zeros_like(ot_ref)

        def qk_setup(h):
            c0 = h * DH
            t0 = c0 // 128
            t1 = (c0 + DH - 1) // 128
            row = lax.broadcasted_iota(jnp.int32, (128, BQ), 0)
            hi = qt_ref[pl.ds(pl.multiple_of(t0 * 128 + 64, 64), 64), :]
            lo = qt_ref[pl.ds(pl.multiple_of(t1 * 128, 128), 64), :]
            qm = jnp.concatenate([lo, hi], axis=0)
            off = c0 - t0 * 128
            msk = ((row - off) & 127) < DH
            qm = jnp.where(msk, qm, jnp.zeros_like(qm))
            return t0 + t1, qm

        def step(h_qk, s_nxt, h_pv, s_cur, m_cur):
            if h_qk is not None:
                kt, qm = qk_setup(h_qk)
                mx = None
            if h_pv is not None:
                c0 = h_pv * DH
                w0 = pl.multiple_of((c0 // 16) * 16, 16)
                off = c0 - w0
                lrow = jnp.where(off == 12, 0, 31)
                row32 = lax.broadcasted_iota(jnp.int32, (32, CK), 0)
                acc = None
                mb = jnp.broadcast_to(m_cur, (CK, BQ))
            for c in range(NC):
                ks = slice(c * CK, (c + 1) * CK)
                if h_qk is not None:
                    s = jnp.dot(kext_ref[kt, ks, :], qm, preferred_element_type=f32)
                    s_nxt[ks, :] = s
                    t = jnp.max(s.reshape(CK // 8, 8, BQ), axis=0)
                    mx = t if mx is None else jnp.maximum(mx, t)
                if h_pv is not None:
                    p = jnp.exp2(s_cur[ks, :] - mb).astype(bf16)
                    r, cc = divmod(c * CK, 512)
                    vt = vt_ref[r, pl.ds(w0, 32), cc:cc + CK]
                    vt = jnp.where(row32 == lrow, jnp.ones_like(vt), vt)
                    t = jnp.dot(vt, p, preferred_element_type=f32)
                    acc = t if acc is None else acc + t
            if h_pv is not None:
                rowq = lax.broadcasted_iota(jnp.int32, (32, BQ), 0)
                l = jnp.sum(jnp.where(rowq == lrow, acc, 0.0), axis=0, keepdims=True)
                o = acc * (1.0 / l)
                valid = (rowq >= off) & (rowq < off + DH)
                ot_ref[pl.ds(w0, 32), :] = jnp.where(valid, o, ot_ref[pl.ds(w0, 32), :])
            if h_qk is not None:
                return jnp.max(mx, axis=0, keepdims=True)

        m = step(0, sa_ref, None, None, None)
        def body(i, m):
            m = step(2 * i + 1, sb_ref, 2 * i, sa_ref, m)
            m = step(2 * i + 2, sa_ref, 2 * i + 1, sb_ref, m)
            return m
        m = lax.fori_loop(0, H // 2 - 1, body, m)
        m = step(H - 1, sb_ref, H - 2, sa_ref, m)
        step(None, None, H - 1, sb_ref, m)

        g = jax.nn.sigmoid(jnp.sum(xq.astype(f32) * gw_ref[...].astype(f32), axis=-1, keepdims=True))
        a = jnp.dot(ot_ref[...].T.astype(bf16), wo_ref[...], preferred_element_type=f32)
        hh = jnp.maximum(jnp.dot(xq, w1_ref[...], preferred_element_type=f32), 0.0).astype(bf16)
        b = jnp.dot(hh, w2_ref[...], preferred_element_type=f32)
        o_ref[...] = (g * a + (1.0 - g) * b).astype(o_ref.dtype)

    @jax.jit
    def fn(A_x, A_wqkv, A_wo, B_x, B_w1, B_w2, gate_w):
        full = lambda shape: pl.BlockSpec(shape, lambda i: (0,) * len(shape))
        out = pl.pallas_call(
            kernel,
            grid=(NQ,),
            in_specs=[full((S, D)), full((D, 3 * D)), full((D, D)), full((D, DFF)), full((DFF, D)), full((1, D))],
            out_specs=pl.BlockSpec((BQ, D), lambda i: (i, 0)),
            out_shape=jax.ShapeDtypeStruct((S, D), A_x.dtype),
            scratch_shapes=[
                pltpu.VMEM((9, S, 128), bf16),
                pltpu.VMEM((S // 512, D, 512), bf16),
                pltpu.VMEM((D, BQ), bf16),
                pltpu.VMEM((S, BQ), f32),
                pltpu.VMEM((S, BQ), f32),
                pltpu.VMEM((D, BQ), f32),
            ],
            compiler_params=pltpu.CompilerParams(
                dimension_semantics=("arbitrary",), vmem_limit_bytes=100 * 2**20),
            name="gmix",
        )(A_x.reshape(S, D), A_wqkv, A_wo, B_w1, B_w2, gate_w.reshape(1, D))
        return out.reshape(1, S, D)
    return fn


pallas_gated_mix__softmax_full_mha__dense_activation_relu__prompt_kernel = make(CK=128)
```

```python
import jax
import jax.numpy as jnp
from jax import lax
import jax.experimental.pallas as pl
import jax.experimental.pallas.tpu as pltpu

S, D, H, DH, DFF = 2048, 640, 32, 20, 1536
LOG2E = 1.4426950408889634
f32, bf16 = jnp.float32, jnp.bfloat16

BQ = 512
CK = 128
NQ = S // BQ
NC = S // CK
NU = NQ * H
MR = 24
LEAD = 2
UNROLL = 14
QPOS = 4
QVB = 2
RC = 256
RO = 128
QM0 = 9 * S // 2


def _dot(a, b):
    return lax.dot_general(a, b, (((1,), (0,)), ((), ())), preferred_element_type=f32)


def _pack(v):
    return pltpu.bitcast(v, jnp.uint32)


def _unpack(v):
    return pltpu.bitcast(v, bf16)


def _blk(r, n):
    return pl.ds(pl.multiple_of(r * n, n), n)


def _dyn(base, off, n):
    return pl.ds(pl.multiple_of(base + off, 8), n)


def _kernel(x_hbm, wqkv_hbm, wo_hbm, w1_hbm, w2_hbm, gw_hbm, o_hbm,
            gw_ref, x_ref, wk_ref, wq_ref, wv_ref, wo_ref, w1_ref, w2_ref, ob_ref,
            kq_ref, vt_ref, qt_ref, s_ref, ot_ref, h0_ref, xsem, wsem, osem):
    def x_copy(r):
        return pltpu.make_async_copy(x_hbm.at[_blk(r, BQ), :], x_ref.at[_blk(r, BQ), :], xsem.at[r])

    def o_copy(r):
        return pltpu.make_async_copy(ob_ref.at[_blk(r, RO), :], o_hbm.at[_blk(r, RO), :], osem.at[r])

    w_copies = [pltpu.make_async_copy(a, b, wsem.at[i]) for i, (a, b) in enumerate([
        (wqkv_hbm.at[:, D:2 * D], wk_ref), (wqkv_hbm.at[:, 0:D], wq_ref), (wqkv_hbm.at[:, 2 * D:3 * D], wv_ref),
        (w1_hbm, w1_ref), (w2_hbm, w2_ref), (wo_hbm, wo_ref), (gw_hbm, gw_ref)])]
    w_copies[0].start()
    x_copy(0).start()
    w_copies[0].wait()

    def k_body(r, _):
        x_copy(r).wait()
        pl.when(r < NQ - 1)(lambda: x_copy(r + 1).start())
        pl.when(r == NQ - 2)(lambda: w_copies[1].start())
        pl.when(r == NQ - 1)(lambda: w_copies[2].start())
        k = _pack(_dot(x_ref[_blk(r, BQ), :], wk_ref[...]).astype(bf16))
        k = [k[:, j * 128:(j + 1) * 128] for j in range(5)]
        lane = lax.broadcasted_iota(jnp.int32, (BQ // 2, 128), 1)
        for j in range(5):
            kq_ref[_blk(2 * j * NQ + r, BQ // 2), :] = k[j]
        for j in range(4):
            kq_ref[_blk((2 * j + 1) * NQ + r, BQ // 2), :] = jnp.where(lane >= 64, k[j], k[j + 1])
        return 0
    lax.fori_loop(0, NQ, k_body, 0)
    w_copies[1].wait()
    w_copies[2].wait()
    for c in w_copies[3:]:
        c.start()

    def qv_body(i, _):
        for r in range(QVB):
            r = i * QVB + r
            xr = x_ref[_blk(r, BQ), :]
            qt_ref[r] = _pack((_dot(xr, wq_ref[...]) * (DH ** -0.5 * LOG2E)).T.astype(bf16))
            vt_ref[r] = _dot(xr, wv_ref[...]).T.astype(bf16).astype(f32)
        return 0
    lax.fori_loop(0, NQ // QVB, qv_body, 0)

    def put_q(u, par, parts):
        w = (u & (H - 1)) * (DH // 2)
        g = w >> 3
        row = lax.broadcasted_iota(jnp.int32, (8, BQ), 0)
        for i in parts:
            t = jnp.zeros((8, BQ), jnp.uint32)
            if i < 2:
                rr = row + ((g + i) * 8 - w)
                t = jnp.where((rr >= 0) & (rr < DH // 2), qt_ref[u >> 5, _blk(g + i, 8), :], t)
            for j in range(4):
                kq_ref[_dyn(((g + i) & 7) * 8, QM0 + par * 256 + j * 64, 8), :] = t[:, j * 128:(j + 1) * 128]

    def qk(u, par, c, mx):
        c0 = (u & (H - 1)) * DH
        kt = (c0 >> 7) + ((c0 + DH - 1) >> 7)
        q0 = QM0 + par * 256
        qm = jnp.concatenate([kq_ref[q0 + j * 64:q0 + (j + 1) * 64, :] for j in range(4)], axis=1)
        s = _dot(_unpack(kq_ref[_dyn(kt * (S // 2), c * CK // 2, CK // 2), :]), _unpack(qm))
        s_ref[par, c * CK:(c + 1) * CK, :] = s
        t = jnp.max(s.reshape(CK // 8, 8, BQ), axis=0)
        return jnp.maximum(mx, t) if c else t

    def step(u, odd, done, mx, nqk=NC, tail=False, filler=None):
        w0 = pl.multiple_of((u & (H - 1)) * DH - 4 * odd, 8)
        lrow = 0 if odd else MR - 1
        rowv = lax.broadcasted_iota(jnp.int32, (MR, CK), 0)
        mb = jnp.broadcast_to(jnp.max(done, axis=0, keepdims=True), (CK, BQ))
        acc = None
        for c in range(NC):
            if QPOS <= c < QPOS + 8 and nqk == NC:
                put_q(u + 2, odd, [c - QPOS])
            p = jnp.exp2(s_ref[odd, c * CK:(c + 1) * CK, :] - mb).astype(bf16)
            r, cc = divmod(c * CK, BQ)
            du, c2 = divmod(c + LEAD, NC)
            for what in ("pv", "qk") if tail and c == NC - 1 else ("qk", "pv"):
                if what == "pv":
                    t = _dot(jnp.where(rowv == lrow, 1.0, vt_ref[r, pl.ds(w0, MR), cc:cc + CK]), p)
                    acc = t if acc is None else acc + t
                elif c < nqk:
                    mx = qk(u + 1 + du, (odd + 1 + du) % 2, c2, mx)
                    if c2 == NC - 1:
                        done = mx
                elif filler is not None:
                    filler(c)
        o = acc * (1.0 / acc[lrow:lrow + 1, :])
        for i in range(BQ // RC):
            b = (u >> 5) * (BQ // RC) + i
            oi = o[:, i * RC:(i + 1) * RC]
            if odd:
                row8 = lax.broadcasted_iota(jnp.int32, (8, RC), 0)
                top = jnp.where(row8 >= 4, oi[0:8], ot_ref[b, pl.ds(w0, 8), :])
                oi = jnp.concatenate([top, oi[8:]], axis=0)
            ot_ref[b, pl.ds(w0, MR), :] = oi
        return done, mx

    def attn_body(i, carry):
        for j in range(UNROLL):
            carry = step(UNROLL * i + j, j % 2, *carry, tail=j == UNROLL - 1)
        return carry

    put_q(0, 0, range(8))
    put_q(1, 1, range(8))
    mx = None
    for c in range(NC):
        mx = qk(0, 0, c, mx)
    done = mx
    for c in range(LEAD):
        mx = qk(1, 1, c, mx)
    nit = (NU - 2) // UNROLL
    carry = lax.fori_loop(0, nit, attn_body, (done, mx))
    for c in w_copies[3:]:
        c.wait()

    def h_head(c):
        if c % 2 == 0:
            rows = slice(c * CK, (c + 2) * CK)
            h0_ref[rows, :] = jnp.maximum(_dot(x_ref[rows, :], w1_ref[:, 0:128]), 0.0).astype(bf16)

    for u in range(nit * UNROLL, NU):
        carry = step(u, u % 2, *carry, nqk=min(NC, max(0, (NU - 1 - u) * NC - LEAD)),
                     filler=h_head if u == NU - 1 else None)

    def out_body(r, _):
        xr = x_ref[_blk(r, RC), :]
        hh = jnp.maximum(_dot(xr, w1_ref[:, 128:]), 0.0).astype(bf16)
        hh = jnp.concatenate([h0_ref[_blk(r, RC), :], hh], axis=1)
        g = jax.nn.sigmoid(jnp.sum(xr.astype(f32) * gw_ref[...].astype(f32)[None, :], axis=-1, keepdims=True))
        a = g * _dot(ot_ref[r].T.astype(bf16), wo_ref[...])
        for i in range(RC // RO):
            sl = slice(i * RO, (i + 1) * RO)
            b = (1.0 - g[sl]) * _dot(hh[sl], w2_ref[...])
            ob_ref[_blk(r * (RC // RO) + i, RO), :] = (a[sl] + b).astype(ob_ref.dtype)
            o_copy(r * (RC // RO) + i).start()
        return 0
    lax.fori_loop(0, S // RC, out_body, 0)
    for r in range(S // RO):
        o_copy(r).wait()


@jax.jit
def pallas_gated_mix__softmax_full_mha__dense_activation_relu__prompt_kernel(
    A_x: jax.Array,
    A_wqkv: jax.Array,
    A_wo: jax.Array,
    B_x: jax.Array,
    B_w1: jax.Array,
    B_w2: jax.Array,
    gate_w: jax.Array,
):
    del B_x
    hbm = pl.BlockSpec(memory_space=pl.ANY)
    out = pl.pallas_call(
        _kernel,
        in_specs=[hbm] * 6,
        out_specs=hbm,
        out_shape=jax.ShapeDtypeStruct((S, D), A_x.dtype),
        scratch_shapes=[
            pltpu.VMEM((D,), bf16),
            pltpu.VMEM((S, D), bf16),
            pltpu.VMEM((D, D), bf16),
            pltpu.VMEM((D, D), bf16),
            pltpu.VMEM((D, D), bf16),
            pltpu.VMEM((D, D), bf16),
            pltpu.VMEM((D, DFF), bf16),
            pltpu.VMEM((DFF, D), bf16),
            pltpu.VMEM((S, D), bf16),
            pltpu.VMEM((QM0 + 512, 128), jnp.uint32),
            pltpu.VMEM((NQ, D, BQ), f32),
            pltpu.VMEM((NQ, D // 2, BQ), jnp.uint32),
            pltpu.VMEM((2, S, BQ), f32),
            pltpu.VMEM((S // RC, D, RC), f32),
            pltpu.VMEM((S, 128), bf16),
            pltpu.SemaphoreType.DMA((NQ,)),
            pltpu.SemaphoreType.DMA((7,)),
            pltpu.SemaphoreType.DMA((S // RO,)),
        ],
        compiler_params=pltpu.CompilerParams(vmem_limit_bytes=100 * 2**20),
        name="gmix",
    )(A_x.reshape(S, D), A_wqkv, A_wo, B_w1, B_w2, gate_w)
    return out.reshape(1, S, D)
```
